```python
import jax
import jax.numpy as jnp

def _softmax(x, axis=-1):
    return jax.nn.softmax(x, axis=axis)
def _gelu(x):
    return jax.nn.gelu(x, approximate=True)
def _silu(x):
    return jax.nn.silu(x)
def _sigmoid(x):
    return jax.nn.sigmoid(x)
def _layernorm(x, axis=-1, eps=1e-5):
    m = jnp.mean(x, axis=axis, keepdims=True)
    v = jnp.var(x, axis=axis, keepdims=True)
    return (x - m) / jnp.sqrt(v + eps)
def _scatter_add(tgt, idx, src, axis=0):
    return tgt.at[idx].add(src)
def _segment_sum(src, seg, n):
    return jax.ops.segment_sum(src, seg, n)
class _Rng:
    def __init__(self, key):
        self._k = key
    def _next(self):
        self._k, sub = jax.random.split(self._k)
        return sub
    def normal(self, shape):
        return jax.random.normal(self._next(), shape, dtype=jnp.bfloat16)
    def randint(self, lo, hi, shape):
        return jax.random.randint(self._next(), shape, lo, hi, dtype=jnp.int32)
    def uniform(self, shape, lo=0.0, hi=1.0):
        return jax.random.uniform(self._next(), shape, jnp.bfloat16, lo, hi)
    def permutation(self, n):
        return jax.random.permutation(self._next(), n)


kernel_name = 'standalone__groupnorm__prompt'

def setup_inputs():
    _rng = _Rng(jax.random.key(int.from_bytes(__import__("os").urandom(4), "little")))
    _w = (lambda a: (lambda t: t.astype(jnp.bfloat16) if jnp.issubdtype(t.dtype, jnp.floating) else t)(jnp.asarray(a)))
    B = 2
    G = 32
    cpg = max(1, 1024 // G)
    C = G * cpg
    H, W = 32, 2048
    return {
        "x": _w((lambda *s: _rng.normal(s) * 0.05)(B, C, H, W)),
        "g": _w((lambda *s: _rng.normal(s) * 0.05)(C) + 1.0),
        "b": _w((lambda *s: _rng.normal(s) * 0.05)(C)),
    }

def reference(x, g, b):
    G = 32
    B, C, H, W = x.shape[0], x.shape[1], x.shape[2], x.shape[3]
    xr = x.reshape(B, G, C // G, H, W)
    mu = xr.mean(axis=(2, 3, 4), keepdims=True)
    var = ((xr - mu) ** 2).mean(axis=(2, 3, 4), keepdims=True)
    xn = (xr - mu) / jnp.sqrt(var + 1e-5)
    xn = xn.reshape(B, C, H, W)
    return xn * g[None, :, None, None] + b[None, :, None, None]
```

```python
import functools

import jax
import jax.numpy as jnp
from jax import lax
import jax.experimental.pallas as pl
import jax.experimental.pallas.tpu as pltpu

G = 32
EPS = 1e-5


def groupnorm(x, g, b, *, phases=(22, 21, 21), ahead=4, r_tail=2, w_tail=2, light=1,
              streams=8, cw=512, nbc=True):
    B, C, H, W = x.shape
    cpg = C // G
    ngroups = B * G
    assert sum(phases) == ngroups
    rows = cpg * H
    bands = rows // (streams * 8)
    ncb = W // cw
    cap = max(phases) * bands
    bands_per_ch = H // 8
    ch_per_stream = cpg // streams
    f32 = jnp.float32

    def kernel(x_hbm, g_hbm, b_hbm, o_hbm, buf, mom, gb_raw, gb_f32, gb, rsem, wsem, psem):
        def hbm_piece(ref, first, it, cb, lo, n):
            return ref.at[first + it // bands, pl.ds(lo, n), it % bands, :, pl.ds(cb * cw, cw)]

        def read_sem(it, cb):
            return rsem.at[(it % ahead) * ncb + cb]

        def start_read(first, it, cb):
            sem = read_sem(it, cb)
            bulk = streams - light
            pltpu.make_async_copy(hbm_piece(x_hbm, first, it, cb, 0, bulk),
                                  buf.at[it, cb, pl.ds(0, bulk)], sem).start(priority=1)
            if light:
                pltpu.make_async_copy(hbm_piece(x_hbm, first, it, cb, bulk, light),
                                      buf.at[it, cb, pl.ds(bulk, light)], sem).start(priority=0)

        def wait_read(it, cb):
            pltpu.make_async_copy(buf.at[it, cb], buf.at[it, cb], read_sem(it, cb)).wait()

        def stats(first, lo, hi, carry, prefetch):
            def body(it, carry):
                mean, m2 = carry
                band = it % bands
                mean = jnp.where(band == 0, 0.0, mean)
                m2 = jnp.where(band == 0, 0.0, m2)
                for cb in range(ncb):
                    wait_read(it, cb)
                    if prefetch:
                        start_read(first, it + ahead, cb)
                    seen = jnp.full((8, 128), band * ncb + cb, jnp.int32).astype(f32)
                    w_new = 1.0 / (seen + 1.0)
                    w_sq = (seen * streams) * w_new
                    w_new = jnp.concatenate([w_new] * (cw // 128), axis=1)
                    w_sq = jnp.concatenate([w_sq] * (cw // 128), axis=1)
                    v = buf[it, cb].astype(f32)
                    mc = jnp.sum(v, axis=0) * (1.0 / streams)
                    d = v - mc
                    delta = mc - mean
                    mean = mean + delta * w_new
                    m2 = m2 + (jnp.sum(d * d, axis=0) + (delta * w_sq) * delta)
                mom[it // bands, 0] = mean
                mom[it // bands, 1] = m2
                return mean, m2
            return lax.fori_loop(lo, hi, body, carry)

        def normalize(first, lo, hi, n_it):
            def group(s, _):
                mean, m2 = mom[s, 0], mom[s, 1]
                mu = jnp.sum(jnp.sum(mean, axis=0, keepdims=True), axis=1, keepdims=True) * (1.0 / (8 * cw))
                d = mean - mu
                t = m2 * (1.0 / (streams * bands * ncb)) + d * d
                var = jnp.sum(jnp.sum(t, axis=0, keepdims=True), axis=1, keepdims=True) * (1.0 / (8 * cw))
                rstd = jnp.broadcast_to(lax.rsqrt(var + EPS), (8, cw))
                mu = jnp.broadcast_to(mu, (8, cw))
                c0 = ((first + s) % G) * cpg

                def body(band, _):
                    it = s * bands + band
                    sem = wsem.at[(it >= n_it - w_tail).astype(jnp.int32)]
                    sc, sh = [], []
                    for j in range(streams):
                        c = c0 + j * ch_per_stream + band // bands_per_ch
                        sc.append(rstd * gb[0, c // 128, c % 128])
                        sh.append(gb[1, c // 128, c % 128])
                    for cb in range(ncb):
                        vs = [buf[it, cb, j].astype(f32) for j in range(streams)]
                        for j in range(streams):
                            buf[it, cb, j] = ((vs[j] - mu) * sc[j] + sh[j]).astype(buf.dtype)
                        pltpu.make_async_copy(buf.at[it, cb], hbm_piece(o_hbm, first, it, cb, 0, streams), sem).start()
                lax.fori_loop(0, bands, body, None)
            lax.fori_loop(lo, hi, group, None)

        def prime(first):
            def body(it, _):
                for cb in range(ncb):
                    start_read(first, it, cb)
            lax.fori_loop(0, ahead, body, None)

        def wait_writes(lo, n, which):
            pltpu.make_async_copy(buf.at[pl.ds(lo, n)], buf.at[pl.ds(lo, n)], wsem.at[which]).wait()

        prime(0)
        params = [pltpu.make_async_copy(g_hbm, gb_raw.at[0], psem.at[0]),
                  pltpu.make_async_copy(b_hbm, gb_raw.at[1], psem.at[1])]
        for p in params:
            p.start()
        for p in params:
            p.wait()
        gb_f32[...] = gb_raw[...].astype(f32)
        to_smem = pltpu.make_async_copy(gb_f32, gb, psem.at[0])
        to_smem.start()

        first = 0
        for ph, n in enumerate(phases):
            n_it = n * bands
            zero = jnp.zeros((8, cw), f32)
            carry = stats(first, 0, n_it - ahead, (zero, zero), True)
            if ph == 0:
                to_smem.wait()
            carry = stats(first, n_it - ahead, n_it - r_tail, carry, False)
            normalize(first, 0, 1, n_it)
            stats(first, n_it - r_tail, n_it, carry, False)
            normalize(first, 1, n, n_it)
            wait_writes(0, n_it - w_tail, 0)
            first += n
            if ph + 1 < len(phases):
                prime(first)
            if w_tail:
                wait_writes(n_it - w_tail, w_tail, 1)

    view = (ngroups, streams, bands, 8, W)
    hbm = pl.BlockSpec(memory_space=pltpu.MemorySpace.HBM)
    out = pl.pallas_call(
        kernel,
        out_shape=jax.ShapeDtypeStruct(view, x.dtype),
        in_specs=[hbm, hbm, hbm],
        out_specs=hbm,
        scratch_shapes=[
            pltpu.VMEM((cap, ncb, streams, 8, cw), x.dtype),
            pltpu.VMEM((max(phases), 2, 8, cw), f32),
            pltpu.VMEM((2, C // 128, 128), g.dtype),
            pltpu.VMEM((2, C // 128, 128), f32),
            pltpu.SMEM((2, C // 128, 128), f32),
            pltpu.SemaphoreType.DMA((ahead * ncb,)),
            pltpu.SemaphoreType.DMA((2,)),
            pltpu.SemaphoreType.DMA((2,)),
        ],
        compiler_params=pltpu.CompilerParams(vmem_limit_bytes=126 * 2**20, disable_bounds_checks=nbc),
    )(x.reshape(view), g.reshape(C // 128, 128), b.reshape(C // 128, 128))
    return out.reshape(x.shape)


@jax.jit
def pallas_standalone__groupnorm__prompt_kernel(x: jax.Array, g: jax.Array, b: jax.Array):
    return groupnorm(x, g, b, nbc=False)
```

```python
import jax
import jax.numpy as jnp
from jax import lax
import jax.experimental.pallas as pl
import jax.experimental.pallas.tpu as pltpu

_GROUPS = 32
_EPS = 1e-5

_BLOCK_GROUPS = 4
_WRITE_GROUPS = 2
_PHASE_BLOCKS = 6
_READ_COLS = 512
_WRITE_COLS = 1024
_READ_AHEAD = 2
_READ_TAIL = 12
_WRITE_HEAD = 8


def _tree_sum(vs):
    while len(vs) > 1:
        vs = [a + b for a, b in zip(vs[::2], vs[1::2])] + vs[len(vs) & ~1:]
    return vs[0]


def _mean(v):
    return jnp.sum(jnp.sum(v, axis=0, keepdims=True), axis=1, keepdims=True) * (1.0 / v.size)


def _divmod(i, n):
    assert n & (n - 1) == 0
    return i >> (n.bit_length() - 1), i & (n - 1)


def _groupnorm(x, g, b, interpret=False):
    B, C, H, W = x.shape
    f32 = jnp.float32
    cpg = C // _GROUPS
    blocks = B * _GROUPS // _BLOCK_GROUPS
    pairs = 2 * _BLOCK_GROUPS
    bands = cpg * H // (4 * 8)
    read_steps = 2 * W // _READ_COLS
    write_steps = W // _WRITE_COLS
    units = _BLOCK_GROUPS // _WRITE_GROUPS
    unit_pairs = 2 * _WRITE_GROUPS
    step_vregs = 2 * _READ_COLS // 128
    phases = pl.cdiv(blocks, _PHASE_BLOCKS)
    head = min(_WRITE_HEAD, bands)
    assert cpg % 4 == 0 and H % 8 == 0 and W % _WRITE_COLS == 0 and C % 128 == 0
    assert bands >= _READ_AHEAD and blocks - (phases - 1) * _PHASE_BLOCKS >= 2
    assert _READ_TAIL <= _READ_AHEAD * read_steps

    def kernel(x_hbm, g_hbm, b_hbm, o_hbm,
               buf, moments, gb_raw, gb_f32, gb, read_sems, write_sems, gb_sems):

        def read_sem(slot, step):
            return read_sems.at[_divmod(slot, _READ_AHEAD)[1] * read_steps + step]

        def start_read(first, slot, step):
            blk, band = _divmod(slot, bands)
            cols = pl.ds(step // 2 * _READ_COLS, _READ_COLS)
            for part, priority in ((pl.ds(0, pairs - 1), 1), (pl.ds(pairs - 1, 1), 0)):
                pltpu.make_async_copy(
                    x_hbm.at[first + blk, part, step % 2, band, :, cols],
                    buf.at[slot, part, step % 2, :, cols],
                    read_sem(slot, step)).start(priority=priority)

        def start_phase(first):
            @pl.loop(0, _READ_AHEAD)
            def _(slot):
                for step in range(read_steps):
                    start_read(first, slot, step)

        def accumulate(first, slot, steps, acc, prefetch):
            blk, band = _divmod(slot, bands)
            acc = list(acc)
            for step in steps:
                cols = pl.ds(step // 2 * _READ_COLS, _READ_COLS)
                landed = buf.at[slot, :, step % 2, :, cols]
                pltpu.make_async_copy(landed, landed, read_sem(slot, step)).wait()
                if prefetch:
                    start_read(first, slot + _READ_AHEAD, step)
                seen = jnp.full((8, 128), band * read_steps + step, jnp.int32).astype(f32)
                w_mean = 1.0 / (seen + 1.0)
                w_sq = seen * step_vregs * w_mean
                for q in range(_BLOCK_GROUPS):
                    mean, m2 = acc[q]
                    if step == 0:
                        mean = jnp.where(band == 0, 0.0, mean)
                        m2 = jnp.where(band == 0, 0.0, m2)
                    v = buf[slot, pl.ds(2 * q, 2), step % 2, :, cols].astype(f32)
                    v = [v[j, :, c:c + 128] for j in range(2) for c in range(0, _READ_COLS, 128)]
                    local = _tree_sum(v) * (1.0 / step_vregs)
                    local_m2 = _tree_sum([(t - local) * (t - local) for t in v])
                    delta = local - mean
                    acc[q] = (mean + delta * w_mean, m2 + (local_m2 + delta * w_sq * delta))
            for q in range(_BLOCK_GROUPS):
                moments[blk * _BLOCK_GROUPS + q, 0] = acc[q][0]
                moments[blk * _BLOCK_GROUPS + q, 1] = acc[q][1]
            return tuple(acc)

        def accumulate_tail(first, slot, lo, hi, acc):
            for k in range(lo // read_steps, pl.cdiv(hi, read_steps)):
                steps = range(max(lo - k * read_steps, 0), min(hi - k * read_steps, read_steps))
                acc = accumulate(first, slot + k, steps, acc, prefetch=False)
            return acc

        def write_copy(first, n, unit, band, step):
            blk, part = _divmod(unit, units)
            part = pl.ds(part * unit_pairs, unit_pairs)
            cols = pl.ds(step * _WRITE_COLS, _WRITE_COLS)
            sem = 0
            if step == write_steps - 1:
                sem = (unit * bands + band == n * units * bands - 1).astype(jnp.int32)
            return pltpu.make_async_copy(
                buf.at[blk * bands + band, part, :, :, cols],
                o_hbm.at[first + blk, part, :, band, :, cols],
                write_sems.at[sem])

        def normalize(first, n, unit, lo, hi):
            blk, part = _divmod(unit, units)
            mus, rstds = [], []
            for q in range(_WRITE_GROUPS):
                mean = moments[unit * _WRITE_GROUPS + q, 0]
                m2 = moments[unit * _WRITE_GROUPS + q, 1]
                mu = _mean(mean)
                var = _mean(m2 * (mean.size / (cpg * H * W)) + (mean - mu) * (mean - mu))
                mus.append(jnp.broadcast_to(mu, (8, _WRITE_COLS)))
                rstds.append(jnp.broadcast_to(lax.rsqrt(var + _EPS), (8, _WRITE_COLS)))
            group = _divmod(first * _BLOCK_GROUPS + unit * _WRITE_GROUPS, _GROUPS)[1]

            @pl.loop(lo, hi)
            def _(band):
                scale, shift = [], []
                for j in range(2 * unit_pairs):
                    channel = group * cpg + j * (cpg // 4) + _divmod(band, H // 8)[0]
                    row, lane = _divmod(channel, 128)
                    scale.append(rstds[j // 4] * gb[0, row, lane])
                    shift.append(gb[1, row, lane])
                for step in range(write_steps):
                    at = [(blk * bands + band, part * unit_pairs + j // 2, j % 2,
                           slice(None), pl.ds(step * _WRITE_COLS, _WRITE_COLS))
                          for j in range(2 * unit_pairs)]
                    for j, v in enumerate([buf[i] for i in at]):
                        y = (v.astype(f32) - mus[j // 4]) * scale[j] + shift[j]
                        buf[at[j]] = y.astype(buf.dtype)
                    write_copy(first, n, unit, band, step).start()

        gb_copies = [pltpu.make_async_copy(src, gb_raw.at[i], gb_sems.at[i])
                     for i, src in enumerate((g_hbm, b_hbm))]
        for copy in gb_copies:
            copy.start()
        start_phase(0)
        for copy in gb_copies:
            copy.wait()
        gb_f32[...] = gb_raw[...].astype(f32)
        to_smem = pltpu.make_async_copy(gb_f32, gb, gb_sems.at[2])
        to_smem.start()

        @pl.loop(0, phases)
        def _(phase):
            first = phase * _PHASE_BLOCKS
            n = jnp.minimum(_PHASE_BLOCKS, blocks - first)

            tail = n * bands - _READ_AHEAD
            zero = jnp.zeros((8, 128), f32)
            acc = lax.fori_loop(
                0, tail,
                lambda slot, acc: accumulate(first, slot, range(read_steps), acc, prefetch=True),
                ((zero, zero),) * _BLOCK_GROUPS)
            pl.when(phase == 0)(to_smem.wait)
            handover = _READ_AHEAD * read_steps - _READ_TAIL
            acc = accumulate_tail(first, tail, 0, handover, acc)

            normalize(first, n, 0, 0, head)
            accumulate_tail(first, tail, handover, handover + _READ_TAIL, acc)

            @pl.loop(0, n * units)
            def _(unit):
                normalize(first, n, unit, jnp.where(unit == 0, head, 0), bands)

            @pl.loop(0, n * units * bands - 1)
            def _(i):
                for step in range(write_steps):
                    write_copy(first, n, *_divmod(i, bands), step).wait()

            for step in range(write_steps - 1):
                write_copy(first, n, n * units - 1, bands - 1, step).wait()
            pl.when(phase + 1 < phases)(lambda: start_phase(first + n))
            write_copy(first, n, n * units - 1, bands - 1, write_steps - 1).wait()

    view = (blocks, pairs, 2, bands, 8, W)
    gb_shape = (C // 128, 128)
    hbm = pl.BlockSpec(memory_space=pltpu.MemorySpace.HBM)
    out = pl.pallas_call(
        kernel,
        out_shape=jax.ShapeDtypeStruct(view, x.dtype),
        in_specs=[hbm, hbm, hbm],
        out_specs=hbm,
        scratch_shapes=[
            pltpu.VMEM((_PHASE_BLOCKS * bands, pairs, 2, 8, W), x.dtype),
            pltpu.VMEM((_PHASE_BLOCKS * _BLOCK_GROUPS, 2, 8, 128), f32),
            pltpu.VMEM((2, *gb_shape), g.dtype),
            pltpu.VMEM((2, *gb_shape), f32),
            pltpu.SMEM((2, *gb_shape), f32),
            pltpu.SemaphoreType.DMA((_READ_AHEAD * read_steps,)),
            pltpu.SemaphoreType.DMA((2,)),
            pltpu.SemaphoreType.DMA((3,)),
        ],
        compiler_params=pltpu.CompilerParams(vmem_limit_bytes=104 * 2**20),
        interpret=interpret,
    )(x.reshape(view), g.reshape(gb_shape), b.reshape(gb_shape))
    return out.reshape(x.shape)


@jax.jit
def pallas_standalone__groupnorm__prompt_kernel(x: jax.Array, g: jax.Array, b: jax.Array):
    return _groupnorm(x, g, b)
```

```python
import jax
import jax.numpy as jnp
from jax import lax
import jax.experimental.pallas as pl
import jax.experimental.pallas.tpu as pltpu

_GROUPS = 32
_EPS = 1e-5

_BLOCK_GROUPS = 4
_PHASE_BLOCKS = 6
_READ_COLS = 512
_WRITE_COLS = 1024
_READ_AHEAD = 2
_READ_TAIL = 12


def _tree_sum(vs):
    while len(vs) > 1:
        vs = [a + b for a, b in zip(vs[::2], vs[1::2])] + vs[len(vs) & ~1:]
    return vs[0]


def _mean(v):
    return jnp.sum(jnp.sum(v, axis=0, keepdims=True), axis=1, keepdims=True) * (1.0 / v.size)


def _divmod(i, n):
    assert n & (n - 1) == 0
    return i >> (n.bit_length() - 1), i & (n - 1)


def _groupnorm(x, g, b, interpret=False):
    B, C, H, W = x.shape
    f32 = jnp.float32
    cpg = C // _GROUPS
    blocks = B * _GROUPS // _BLOCK_GROUPS
    pairs = 2 * _BLOCK_GROUPS
    bands = cpg * H // (4 * 8)
    read_steps = 2 * W // _READ_COLS
    write_steps = W // _WRITE_COLS
    step_vregs = 2 * _READ_COLS // 128
    phases = pl.cdiv(blocks, _PHASE_BLOCKS)
    assert cpg % 4 == 0 and H % 8 == 0 and W % _WRITE_COLS == 0 and C % 128 == 0
    assert bands >= _READ_AHEAD and blocks // phases >= 3
    assert _READ_TAIL <= _READ_AHEAD * read_steps

    def kernel(x_hbm, g_hbm, b_hbm, o_hbm,
               buf, moments, gb_raw, gb_f32, gb, read_sems, write_sems, gb_sems):

        def read_sem(slot, step):
            return read_sems.at[_divmod(slot, _READ_AHEAD)[1] * read_steps + step]

        def start_read(first, slot, step):
            blk, band = _divmod(slot, bands)
            cols = pl.ds(step // 2 * _READ_COLS, _READ_COLS)
            for lo, size, priority in ((0, pairs - 1, 1), (pairs - 1, 1, 0)):
                pltpu.make_async_copy(
                    x_hbm.at[pl.ds((first + blk) * pairs + lo, size), step % 2, band, :, cols],
                    buf.at[pl.ds(blk * pairs + lo, size), step % 2, band, :, cols],
                    read_sem(slot, step)).start(priority=priority)

        def start_phase(first):
            @pl.loop(0, _READ_AHEAD)
            def _(slot):
                for step in range(read_steps):
                    start_read(first, slot, step)

        def accumulate(first, slot, steps, acc, prefetch):
            blk, band = _divmod(slot, bands)
            acc = list(acc)
            for step in steps:
                cols = pl.ds(step // 2 * _READ_COLS, _READ_COLS)
                landed = buf.at[pl.ds(blk * pairs, pairs), step % 2, band, :, cols]
                pltpu.make_async_copy(landed, landed, read_sem(slot, step)).wait()
                if prefetch:
                    start_read(first, slot + _READ_AHEAD, step)
                seen = jnp.full((8, 128), band * read_steps + step, jnp.int32).astype(f32)
                w_mean = 1.0 / (seen + 1.0)
                w_sq = seen * step_vregs * w_mean
                for q in range(_BLOCK_GROUPS):
                    mean, m2 = acc[q]
                    if step == 0:
                        mean = jnp.where(band == 0, 0.0, mean)
                        m2 = jnp.where(band == 0, 0.0, m2)
                    v = buf[pl.ds(blk * pairs + 2 * q, 2), step % 2, band, :, cols].astype(f32)
                    v = [v[j, :, c:c + 128] for j in range(2) for c in range(0, _READ_COLS, 128)]
                    local = _tree_sum(v) * (1.0 / step_vregs)
                    local_m2 = _tree_sum([(t - local) * (t - local) for t in v])
                    delta = local - mean
                    acc[q] = (mean + delta * w_mean, m2 + (local_m2 + delta * w_sq * delta))
            for q in range(_BLOCK_GROUPS):
                moments[blk * _BLOCK_GROUPS + q, 0] = acc[q][0]
                moments[blk * _BLOCK_GROUPS + q, 1] = acc[q][1]
            return tuple(acc)

        def accumulate_tail(first, slot, lo, hi, acc):
            for k in range(lo // read_steps, pl.cdiv(hi, read_steps)):
                steps = range(max(lo - k * read_steps, 0), min(hi - k * read_steps, read_steps))
                acc = accumulate(first, slot + k, steps, acc, prefetch=False)
            return acc

        def write_copy(first, n, pair, size, band, step):
            cols = pl.ds(step * _WRITE_COLS, _WRITE_COLS)
            sem = 0
            if step == write_steps - 1:
                sem = ((pair + size == n * pairs) & (band == bands - 1)).astype(jnp.int32)
            return pltpu.make_async_copy(
                buf.at[pl.ds(pair, size), :, band, :, cols],
                o_hbm.at[pl.ds(first * pairs + pair, size), :, band, :, cols],
                write_sems.at[sem])

        def normalize(first, n, pair, size):
            mus, rstds = [], []
            for p in range(size):
                mean = moments[(pair + p) >> 1, 0]
                m2 = moments[(pair + p) >> 1, 1]
                mu = _mean(mean)
                var = _mean(m2 * (mean.size / (cpg * H * W)) + (mean - mu) * (mean - mu))
                mus.append(jnp.broadcast_to(mu, (8, _WRITE_COLS)))
                rstds.append(jnp.broadcast_to(lax.rsqrt(var + _EPS), (8, _WRITE_COLS)))

            @pl.loop(0, bands)
            def _(band):
                scale, shift = [], []
                for j in range(2 * size):
                    stream = _divmod(2 * (first * pairs + pair) + j, 4 * _GROUPS)[1]
                    row, lane = _divmod(stream * (cpg // 4) + _divmod(band, H // 8)[0], 128)
                    scale.append(rstds[j // 2] * gb[0, row, lane])
                    shift.append(gb[1, row, lane])
                for step in range(write_steps):
                    cols = pl.ds(step * _WRITE_COLS, _WRITE_COLS)
                    at = [(pair + j // 2, j % 2, band, slice(None), cols) for j in range(2 * size)]
                    for j, v in enumerate([buf[i] for i in at]):
                        y = (v.astype(f32) - mus[j // 2]) * scale[j] + shift[j]
                        buf[at[j]] = y.astype(buf.dtype)
                    write_copy(first, n, pair, size, band, step).start()

        def wait_writes(first, n, pair, size, count):
            @pl.loop(0, count)
            def _(i):
                unit, band = _divmod(i, bands)
                for step in range(write_steps):
                    write_copy(first, n, pair + unit * size, size, band, step).wait()

        gb_copies = [pltpu.make_async_copy(src, gb_raw.at[i], gb_sems.at[i])
                     for i, src in enumerate((g_hbm, b_hbm))]
        for copy in gb_copies:
            copy.start()
        start_phase(0)
        for copy in gb_copies:
            copy.wait()
        gb_f32[...] = gb_raw[...].astype(f32)
        to_smem = pltpu.make_async_copy(gb_f32, gb, gb_sems.at[2])
        to_smem.start()

        @pl.loop(0, phases)
        def _(phase):
            first = phase * (blocks // phases) + jnp.minimum(phase, blocks % phases)
            n = blocks // phases + (phase < blocks % phases).astype(jnp.int32)

            tail = n * bands - _READ_AHEAD
            zero = jnp.zeros((8, 128), f32)
            acc = lax.fori_loop(
                0, tail,
                lambda slot, acc: accumulate(first, slot, range(read_steps), acc, prefetch=True),
                ((zero, zero),) * _BLOCK_GROUPS)
            pl.when(phase == 0)(to_smem.wait)
            handover = _READ_AHEAD * read_steps - _READ_TAIL
            acc = accumulate_tail(first, tail, 0, handover, acc)

            fours = lax.rem(n * pairs - 1, 3) + 1
            threes = lax.div(n * pairs - 4 * fours, 3)
            pl.loop(0, fours)(lambda i: normalize(first, n, 4 * i, 4))
            accumulate_tail(first, tail, handover, handover + _READ_TAIL, acc)
            pl.loop(0, threes)(lambda i: normalize(first, n, 4 * fours + 3 * i, 3))

            wait_writes(first, n, 0, 4, fours * bands)
            wait_writes(first, n, 4 * fours, 3, threes * bands - 1)
            for step in range(write_steps - 1):
                write_copy(first, n, n * pairs - 3, 3, bands - 1, step).wait()
            pl.when(phase + 1 < phases)(lambda: start_phase(first + n))
            write_copy(first, n, n * pairs - 3, 3, bands - 1, write_steps - 1).wait()

    view = (blocks * pairs, 2, bands, 8, W)
    gb_shape = (C // 128, 128)
    hbm = pl.BlockSpec(memory_space=pltpu.MemorySpace.HBM)
    out = pl.pallas_call(
        kernel,
        out_shape=jax.ShapeDtypeStruct(view, x.dtype),
        in_specs=[hbm, hbm, hbm],
        out_specs=hbm,
        scratch_shapes=[
            pltpu.VMEM((_PHASE_BLOCKS * pairs, *view[1:]), x.dtype),
            pltpu.VMEM((_PHASE_BLOCKS * _BLOCK_GROUPS, 2, 8, 128), f32),
            pltpu.VMEM((2, *gb_shape), g.dtype),
            pltpu.VMEM((2, *gb_shape), f32),
            pltpu.SMEM((2, *gb_shape), f32),
            pltpu.SemaphoreType.DMA((_READ_AHEAD * read_steps,)),
            pltpu.SemaphoreType.DMA((2,)),
            pltpu.SemaphoreType.DMA((3,)),
        ],
        compiler_params=pltpu.CompilerParams(vmem_limit_bytes=104 * 2**20),
        interpret=interpret,
    )(x.reshape(view), g.reshape(gb_shape), b.reshape(gb_shape))
    return out.reshape(x.shape)


@jax.jit
def pallas_standalone__groupnorm__prompt_kernel(x: jax.Array, g: jax.Array, b: jax.Array):
    return _groupnorm(x, g, b)
```
